```python
import jax
import jax.numpy as jnp

def _softmax(x, axis=-1):
    return jax.nn.softmax(x, axis=axis)

def _gelu(x):
    return jax.nn.gelu(x, approximate=True)

def _silu(x):
    return jax.nn.silu(x)

def _sigmoid(x):
    return jax.nn.sigmoid(x)

def _layernorm(x, axis=-1, eps=1e-05):
    m = jnp.mean(x, axis=axis, keepdims=True)
    v = jnp.var(x, axis=axis, keepdims=True)
    return (x - m) / jnp.sqrt(v + eps)

def _scatter_add(tgt, idx, src, axis=0):
    return tgt.at[idx].add(src)

def _segment_sum(src, seg, n):
    return jax.ops.segment_sum(src, seg, n)

class _Rng:

    def __init__(self, key):
        self._k = key

    def _next(self):
        self._k, sub = jax.random.split(self._k)
        return sub

    def normal(self, shape):
        return jax.random.normal(self._next(), shape, dtype=jnp.bfloat16)

    def randint(self, lo, hi, shape):
        return jax.random.randint(self._next(), shape, lo, hi, dtype=jnp.int32)

    def uniform(self, shape, lo=0.0, hi=1.0):
        return jax.random.uniform(self._next(), shape, jnp.bfloat16, lo, hi)

    def permutation(self, n):
        return jax.random.permutation(self._next(), n)
kernel_name = 'adaLN_cond__sliding_block_cached__mixer_s_mlp__decode'

def setup_inputs():
    _rng = _Rng(jax.random.key(int.from_bytes(__import__("os").urandom(4), "little")))
    _w = lambda a: (lambda t: t.astype(jnp.bfloat16) if jnp.issubdtype(t.dtype, jnp.floating) else t)(jnp.asarray(a))

    def _A_setup():
        B, Sq, D = (1, 1, 448)
        Hq, Hkv, Sk, Dh = (16, 8, 65536, 256)
        assert Hq % Hkv == 0, (Hq, Hkv)
        return {'x': _w((lambda *s: _rng.normal(s) * 0.05)(B, Sq, D)), 'k_cache': _w((lambda *s: _rng.normal(s) * 0.05)(B, Hkv, Sk, Dh)), 'v_cache': _w((lambda *s: _rng.normal(s) * 0.05)(B, Hkv, Sk, Dh)), 'wq': _w((lambda *s: _rng.normal(s) * 0.05)(D, Hq * Dh) * D ** (-0.5)), 'wo': _w((lambda *s: _rng.normal(s) * 0.05)(Hq * Dh, D) * (Hq * Dh) ** (-0.5))}
    _A_in = _A_setup()

    def _B_setup():
        B, S, D, F = (1, 1, 448, 1792)
        return {'x': _w((lambda *s: _rng.normal(s) * 0.05)(B, S, D)), 'w1': _w((lambda *s: _rng.normal(s) * 0.05)(D, D) * D ** (-0.5)), 'w2': _w((lambda *s: _rng.normal(s) * 0.05)(D, D) * D ** (-0.5)), 'w3': _w((lambda *s: _rng.normal(s) * 0.05)(D, F) * D ** (-0.5)), 'w4': _w((lambda *s: _rng.normal(s) * 0.05)(F, D) * F ** (-0.5))}
    _B_in = _B_setup()
    return {'A_x': _A_in['x'], 'A_k_cache': _A_in['k_cache'], 'A_v_cache': _A_in['v_cache'], 'A_wq': _A_in['wq'], 'A_wo': _A_in['wo'], 'B_x': _B_in['x'], 'B_w1': _B_in['w1'], 'B_w2': _B_in['w2'], 'B_w3': _B_in['w3'], 'B_w4': _B_in['w4'], 'c': _w((lambda *s: _rng.normal(s) * 0.05)(1, 448)), 'w_mod': _w((lambda *s: _rng.normal(s) * 0.05)(448, 6 * 448) * 448 ** (-0.5))}

def reference(A_x, A_k_cache, A_v_cache, A_wq, A_wo, B_x, B_w1, B_w2, B_w3, B_w4, c, w_mod):

    def _A_ref(x, k_cache, v_cache, wq, wo):
        B, Sq, D = x.shape
        Hq, Dh = (16, 256)
        Hkv, Sk = (k_cache.shape[1], k_cache.shape[2])
        W = min(4096, max(256, Sk // 4))
        rep = Hq // Hkv
        q = (lambda x, *d: x.transpose(*d))((x @ wq).reshape(B, Sq, Hq, Dh), 0, 2, 1, 3)
        k = jnp.repeat(k_cache[:, :, Sk - W:, :], rep, axis=1)
        v = jnp.repeat(v_cache[:, :, Sk - W:, :], rep, axis=1)
        scores = jnp.einsum('bhqd,bhkd->bhqk', q, k) * Dh ** (-0.5)
        p = _softmax(scores, axis=-1)
        o = jnp.einsum('bhqk,bhkd->bhqd', p, v)
        return (lambda x, *d: x.transpose(*d))(o, 0, 2, 1, 3).reshape(B, Sq, Hq * Dh) @ wo

    def _B_ref(x, w1, w2, w3, w4):
        B, S, D = x.shape
        h = _gelu(_layernorm(x, axis=-1) @ w1)
        c = D // 4
        g0 = jnp.pad(h[:, :, 0 * c:1 * c], ((0, 0), (1, 0), (0, 0)))[:, :S, :]
        g1 = jnp.pad(h[:, :, 1 * c:2 * c], ((0, 0), (0, 1), (0, 0)))[:, 1:, :]
        g2 = jnp.pad(h[:, :, 2 * c:3 * c], ((0, 0), (2, 0), (0, 0)))[:, :S, :]
        g3 = jnp.pad(h[:, :, 3 * c:], ((0, 0), (0, 2), (0, 0)))[:, 2:, :]
        hs = jnp.concatenate([g0, g1, g2, g3], axis=-1) @ w2
        x1 = x + hs
        h2 = _gelu(_layernorm(x1, axis=-1) @ w3) @ w4
        return x1 + h2
    x = A_x
    mod = (_silu(c) @ w_mod).reshape(c.shape[0], 6, 1, -1)
    sa, ca, ga, sb, cb, gb = (mod[:, 0].copy(), mod[:, 1].copy(), mod[:, 2].copy(), mod[:, 3].copy(), mod[:, 4].copy(), mod[:, 5].copy())
    h = _layernorm(x, axis=-1) * (1 + ca) + sa
    x = x + ga * _A_ref(h, A_k_cache, A_v_cache, A_wq, A_wo)
    h = _layernorm(x, axis=-1) * (1 + cb) + sb
    x = x + gb * _B_ref(h, B_w1, B_w2, B_w3, B_w4)
    return x
```

```python
import jax
import jax.numpy as jnp
from jax import lax
from jax.experimental import pallas as pl
from jax.experimental.pallas import tpu as pltpu

D, F = 448, 1792
HQ, HKV, DH = 16, 8, 256
EPS = 1e-5
BF16, F32 = jnp.bfloat16, jnp.float32
ROWS = 8
ROW_TILES = D // 8
PAGE = 64
PAGE_TILES = 16
STRIDE = 17
SHORT = 1
HEAD_START = 26
GATE_COL = 18 * 128
GATE_BLOCKS = ((0, 320), (320, 112), (432, 16))
W4_BLOCKS = ((0, 256), (256, 128), (384, 64))
V7_FIRST, W4_FIRST = 16, 16
AT = dict(ctx=32, sc=60, ctx6=24, sc7=56, ctx7=72, ln=94)

S_X, S_C, S_WM, S_WQ, S_WO, S_W3, S_K, S_V, S_W4, S_GATE, SEMS = 0, 1, 2, 3, 4, 5, 6, 14, 22, 25, 28


def _layernorm(x):
    d = x - jnp.sum(x, axis=-1, keepdims=True) * (1.0 / D)
    return d * lax.rsqrt(jnp.sum(d * d, axis=-1, keepdims=True) * (1.0 / D) + EPS)


def _dot(a, b):
    return lax.dot_general(a, b, (((1,), (0,)), ((), ())), preferred_element_type=F32)


def _dot_t(a, b):
    return lax.dot_general(a, b, (((1,), (1,)), ((), ())), preferred_element_type=F32)


def _ds(start, size, align):
    return pl.ds(start if isinstance(start, int) else pl.multiple_of(start, align), size)


def _scatter(pages):
    return [pages[p] for i in range(STRIDE) for p in range(4 * i % STRIDE, len(pages), STRIDE)]


def _block(blocks, row):
    return sum(row >= first for first, _ in blocks[1:])


def _kernel(x_hbm, c_hbm, wm_hbm, wq_hbm, k_hbm, v_hbm, wo_hbm, w3_hbm, w4_hbm, out_hbm,
            x_ref, c_ref, wm_ref, wg_ref, wq_ref, k_ref, v_ref, wo_ref, w3_ref, w4_ref,
            q_ref, s_ref, max_ref, attn_ref, mod_ref, ct_ref, out_ref, sems):
    window = k_ref.shape[1]
    first_key = k_hbm.shape[2] - window

    def cache_pages(hbm, ref, sem):
        short = SHORT * PAGE // 2

        def head(h):
            def copy(row, rows):
                return pltpu.make_async_copy(hbm.at[0, h, _ds(first_key + row, rows, PAGE // 2)],
                                             ref.at[h, _ds(row, rows, PAGE // 2)], sems.at[sem + h])

            def page(j):
                if short and isinstance(j, int) and j == 0:
                    return [copy(0, PAGE - short), copy(window - short, short)]
                return [copy((j * STRIDE & 63) * PAGE - short, PAGE)]
            return page
        return head

    def wide_pages(hbm, ref, sem):
        width = ref.shape[1] // 128
        pages = []
        for start in range(-SHORT * PAGE_TILES // 2, ROW_TILES * width, PAGE_TILES):
            lo, hi = max(start, 0), min(start + PAGE_TILES, ROW_TILES * width)
            pages.append([])
            while lo < hi:
                row, col = divmod(lo, width)
                n = min(hi - lo, width - col)
                at = (pl.ds(row * 8, 8), pl.ds(col * 128, n * 128))
                pages[-1].append(pltpu.make_async_copy(hbm.at[at], ref.at[at], sems.at[sem]))
                lo += n
        return _scatter(pages)

    def row_pages(hbm, ref, sem, rows=8, col=0):
        return [[pltpu.make_async_copy(hbm.at[pl.ds(r, rows), pl.ds(col, ref.shape[1])],
                                       ref.at[pl.ds(r, rows)], sems.at[sem(r)])] for r in range(0, D, rows)]

    keys, values = cache_pages(k_hbm, k_ref, S_K), cache_pages(v_hbm, v_ref, S_V)
    wq, wo = wide_pages(wq_hbm, wq_ref, S_WQ), wide_pages(wo_hbm, wo_ref, S_WO)
    wm = _scatter(row_pages(wm_hbm, wm_ref, lambda r: S_WM))
    w3 = _scatter(row_pages(w3_hbm, w3_ref, lambda r: S_W3))
    w4 = row_pages(w4_hbm, w4_ref, lambda r: S_W4 + _block(W4_BLOCKS, r))
    w4 = [w4[(r0 + half * n // 2) // 8 + i] for r0, n in W4_BLOCKS for i in range(n // 16) for half in range(2)]
    wg = row_pages(wm_hbm, wg_ref, lambda r: S_GATE + _block(GATE_BLOCKS, r), 16, GATE_COL)
    x_copy = pltpu.make_async_copy(x_hbm, x_ref, sems.at[S_X])
    c_copy = pltpu.make_async_copy(c_hbm, c_ref, sems.at[S_C])

    def enqueue(first, second=()):
        for copy in first:
            copy.start(priority=1)
        for copy in second:
            copy.start(priority=0)

    def enqueue_all(first, second, work):
        for j, page in enumerate(first):
            lo, hi = j * len(second) // len(first), (j + 1) * len(second) // len(first)
            enqueue(page, [copy for other in second[lo:hi] for copy in other])
            if j in work:
                work[j]()

    def stream(first, second, lo, hi):
        if lo == 0:
            for j in range(4):
                enqueue(first(j), second(j))
            lo = 4

        def body(i, carry):
            for k in range(4):
                enqueue(first(i * 4 + k), second(i * 4 + k))
            return carry
        lax.fori_loop(lo // 4, hi // 4, body, None)

    def landed(ref, sem):
        pltpu.make_async_copy(ref, ref, sems.at[sem]).wait()

    even = (lax.broadcasted_iota(jnp.int32, (ROWS, DH), 0) & 1) == 0

    def condition():
        c_copy.wait()
        landed(wm_ref, S_WM)
        c = jnp.broadcast_to(c_ref[...].astype(F32), (ROWS, D))
        c = (c * jax.nn.sigmoid(c)).astype(BF16)

        def body(i, carry):
            cols = _ds(i * 768, 768, 768)
            s_ref[0, :, cols] = _dot(c, wm_ref[:, cols])
            return carry
        lax.fori_loop(0, GATE_COL // 768, body, None)
        s_ref[0, :, GATE_COL:6 * D] = jnp.zeros((ROWS, 6 * D - GATE_COL), F32)
        for g in range(6):
            mod_ref[g] = s_ref[0, :, g * D:(g + 1) * D]
        s_ref[1, :, :512] = jnp.zeros((ROWS, 512), F32)
        s_ref[1, :, :D] = c.astype(F32)
        for t in range(0, 512, 128):
            ct_ref[t:t + 128] = jnp.broadcast_to(s_ref[1, 0:1, t:t + 128], (128, 128)).T

    def queries():
        x_copy.wait()
        landed(wq_ref, S_WQ)
        x = jnp.broadcast_to(x_ref[0].astype(F32), (ROWS, D))
        h_in = (_layernorm(x) * (1.0 + mod_ref[1]) + mod_ref[0]).astype(BF16)

        def body(h, carry):
            q = _dot(h_in, wq_ref[:, _ds(h * 2 * DH, 2 * DH, 2 * DH)]) * DH ** -0.5
            q_ref[h] = jnp.where(even, q[:, :DH], q[:, DH:])
            return carry
        lax.fori_loop(0, HKV, body, None)
        attn_ref[...] = jnp.zeros((ROWS, D), F32)

    def scores(h):
        landed(k_ref.at[h], S_K + h)
        s = _dot_t(q_ref[h].astype(BF16), k_ref[h])
        s_ref[h] = s
        m = s[:, :128]
        for t in range(128, window, 128):
            m = jnp.maximum(m, s[:, t:t + 128])
        max_ref[h] = jnp.broadcast_to(jnp.max(m, axis=-1, keepdims=True), (ROWS, 128))

    def context(h):
        landed(v_ref.at[h], S_V + h)
        p = jnp.exp(s_ref[h] - jnp.concatenate([max_ref[h]] * (window // 128), axis=1))
        total = p[:, :128]
        for t in range(128, window, 128):
            total = total + p[:, t:t + 128]
        o = _dot(p.astype(BF16), v_ref[h]) / jnp.sum(total, axis=-1, keepdims=True)
        o = jnp.concatenate([jnp.where(even, o, 0.0), jnp.where(even, 0.0, o)], axis=1).astype(BF16)
        attn_ref[...] += _dot_t(o, wo_ref[:, _ds(h * 2 * DH, 2 * DH, 2 * DH)])

    def residual():
        attn = attn_ref[...]
        x = jnp.broadcast_to(x_ref[0].astype(F32), (ROWS, D))
        x = x + mod_ref[2] * (attn + pltpu.roll(attn, 1, 0))
        h_mlp = _layernorm(x) * (1.0 + mod_ref[4]) + mod_ref[3]
        mod_ref[0], mod_ref[1], mod_ref[2] = x, h_mlp, _layernorm(h_mlp)

    k0 = [keys(0)(j) for j in range(64)]
    for page in k0[:HEAD_START]:
        enqueue(page)
    split = (HEAD_START + len(wq) + len(wo) - len(wm) - len(k0)) // 2
    enqueue_all(wm + wo[:split + 1] + k0[HEAD_START:], [[c_copy, x_copy]] + wq + wo[split + 1:], {})
    condition()

    def period(h, carry):
        stream(keys(h + 1), values(h), 0, AT["ctx"])
        pl.when(h == 0)(queries)
        pl.when(h == 1)(lambda: landed(wo_ref, S_WO))
        pl.when(h > 0)(lambda: context(h - 1))
        stream(keys(h + 1), values(h), AT["ctx"], AT["sc"])
        scores(h)
        stream(keys(h + 1), values(h), AT["sc"], 64)
        return carry
    lax.fori_loop(0, HKV - 1, period, None)

    v7 = [values(7)(j) for j in range(64)]
    shared = len(w4) - 2 * W4_FIRST
    enqueue_all(v7[64 - V7_FIRST:] + w3 + w4[shared::2] + wg,
                v7[:64 - V7_FIRST] + w4[:shared] + w4[shared + 1::2],
                {AT["ctx6"]: lambda: context(6), AT["sc7"]: lambda: scores(7),
                 AT["ctx7"]: lambda: context(7), AT["ln"]: residual})

    landed(w3_ref, S_W3)
    hidden = jax.nn.gelu(_dot(mod_ref[2].astype(BF16), w3_ref[...]), approximate=True).astype(BF16)
    for i, (r0, n) in enumerate(W4_BLOCKS):
        landed(w4_ref.at[pl.ds(r0, n)], S_W4 + i)
        mod_ref[1, :, r0:r0 + n] += _dot_t(hidden, w4_ref[r0:r0 + n, :])
    y = mod_ref[1]
    out = mod_ref[0] + mod_ref[5] * y

    gate = [0.0] * 3
    for i, (r0, n) in enumerate(GATE_BLOCKS):
        landed(wg_ref.at[pl.ds(r0, n)], S_GATE + i)
        for r in range(r0, r0 + n, 16):
            for t in range(3):
                part = ct_ref[r:r + 16] * wg_ref[r:r + 16, t * 128:(t + 1) * 128].astype(F32)
                gate[t] = gate[t] + (part[:8] + part[8:])
    low = lax.broadcasted_iota(jnp.int32, (ROWS, 128), 1) < 64
    gate = [pltpu.roll(g, 64, 1) for g in gate]
    gate = [jnp.where(low, a, b) for a, b in zip([0.0] + gate, gate + [0.0])]
    gate = jnp.concatenate([jnp.sum(g, axis=0, keepdims=True) for g in gate], axis=1)
    out_ref[0] = (out[0:1] + gate[:, :D] * y[0:1]).astype(BF16)
    store = pltpu.make_async_copy(out_ref, out_hbm, sems.at[S_X])
    store.start()
    store.wait()


@jax.jit
def pallas_adaLN_cond__sliding_block_cached__mixer_s_mlp__decode_kernel(
    A_x: jax.Array,
    A_k_cache: jax.Array,
    A_v_cache: jax.Array,
    A_wq: jax.Array,
    A_wo: jax.Array,
    B_x: jax.Array,
    B_w1: jax.Array,
    B_w2: jax.Array,
    B_w3: jax.Array,
    B_w4: jax.Array,
    c: jax.Array,
    w_mod: jax.Array,
):
    keys = A_k_cache.shape[2]
    window = min(4096, max(256, keys // 4))
    assert A_x.shape == (1, 1, D) and A_k_cache.shape == (1, HKV, keys, DH) and window == 4096
    hbm = pl.BlockSpec(memory_space=pltpu.HBM)
    return pl.pallas_call(
        _kernel,
        out_shape=jax.ShapeDtypeStruct(A_x.shape, A_x.dtype),
        in_specs=[hbm] * 9,
        out_specs=hbm,
        scratch_shapes=[
            pltpu.VMEM((1, 1, D), BF16),
            pltpu.VMEM((1, D), BF16),
            pltpu.VMEM((D, GATE_COL), BF16),
            pltpu.VMEM((D, 6 * D - GATE_COL), BF16),
            pltpu.VMEM((D, HQ * DH), BF16),
            pltpu.VMEM((HKV, window, DH), BF16),
            pltpu.VMEM((HKV, window, DH), BF16),
            pltpu.VMEM((D, HQ * DH), BF16),
            pltpu.VMEM((D, F), BF16),
            pltpu.VMEM((D, F), BF16),
            pltpu.VMEM((HKV, ROWS, DH), F32),
            pltpu.VMEM((HKV, ROWS, window), F32),
            pltpu.VMEM((HKV, ROWS, 128), F32),
            pltpu.VMEM((ROWS, D), F32),
            pltpu.VMEM((6, ROWS, D), F32),
            pltpu.VMEM((512, 128), F32),
            pltpu.VMEM((1, 1, D), BF16),
            pltpu.SemaphoreType.DMA((SEMS,)),
        ],
        compiler_params=pltpu.CompilerParams(
            vmem_limit_bytes=100 * 2**20,
            disable_semaphore_checks=True,
        ),
        name="adaln_decode",
    )(A_x, c, w_mod, A_wq, A_k_cache, A_v_cache, A_wo.T, B_w3, B_w4.T)
```

```python
import jax
import jax.numpy as jnp
from jax import lax
from jax.experimental import pallas as pl
from jax.experimental.pallas import tpu as pltpu

D, F = 448, 1792
HQ, HKV, DH = 16, 8, 256
EPS = 1e-5
BF16, F32 = jnp.bfloat16, jnp.float32
ROWS = 8
ROW_TILES = D // 8
QUARTER = 32
STREAMS = 5
UNIT_STRIDE = 13
PIECES_1 = ((-2, 1, 0), (1, 1, 3), (-1, 2, 1))
PIECES_0 = ((-1, 2, 1), (-2, 1, -1), (1, 1, 2))
ROW_STRIDE = 17
HEAD_START = 26
GATE_COL = 18 * 128
GATE_BLOCKS = ((0, 320), (320, 112), (432, 16))
W4_BLOCKS = ((0, 256), (256, 128), (384, 64))
V_FIRST = 84
W4_FIRST = 20
AT = dict(a=12, b=22, d=48, c4=40, c5=64, s6=84, s7=104, c6=146, c7=160, ln=172)

S_X, S_C, S_WM, S_WQ, S_WO, S_W3, S_K, S_V, S_W4, S_GATE, SEMS = 0, 1, 2, 3, 4, 5, 6, 14, 22, 25, 28


def _layernorm(x):
    d = x - jnp.sum(x, axis=-1, keepdims=True) * (1.0 / D)
    return d * lax.rsqrt(jnp.sum(d * d, axis=-1, keepdims=True) * (1.0 / D) + EPS)


def _dot(a, b):
    return lax.dot_general(a, b, (((1,), (0,)), ((), ())), preferred_element_type=F32)


def _dot_t(a, b):
    return lax.dot_general(a, b, (((1,), (1,)), ((), ())), preferred_element_type=F32)


def _ds(start, size, align):
    return pl.ds(start if isinstance(start, int) else pl.multiple_of(start, align), size)


def _scatter(copies):
    return [copies[p] for i in range(ROW_STRIDE) for p in range(4 * i % ROW_STRIDE, len(copies), ROW_STRIDE)]


def _block(blocks, row):
    return sum(row >= first for first, _ in blocks[1:])


def _kernel(x_hbm, c_hbm, wm_hbm, wq_hbm, k_hbm, v_hbm, wo_hbm, w3_hbm, w4_hbm, out_hbm,
            x_ref, c_ref, wm_ref, wg_ref, wq_ref, k_ref, v_ref, wo_ref, w3_ref, w4_ref,
            q_ref, s_ref, max_ref, attn_ref, mod_ref, ct_ref, out_ref, sems):
    window = k_ref.shape[1]
    first_key = k_hbm.shape[2] - window

    def cache_copies(hbm, ref, sem, pair, pieces):
        def copy(h, quarter, n):
            row, rows = (quarter & 127) * QUARTER, n * QUARTER
            return pltpu.make_async_copy(hbm.at[0, h, _ds(first_key + row, rows, QUARTER)],
                                         ref.at[h, _ds(row, rows, QUARTER)], sems.at[sem + h])

        def step(i):
            copies = []
            for first, n, delay in pieces:
                unit = (i + 64 - delay) * UNIT_STRIDE & 63
                h, quarter = 2 * pair + (unit >> 5), 4 * (unit & 31) + 128 + first
                if n == 2 and isinstance(i, int) and unit & 31 == 0:
                    copies.append([copy(h, quarter, 1), copy(h, quarter + 1, 1)])
                else:
                    copies.append([copy(h, quarter, n)])
            return copies
        return step

    def wide_copies(hbm, ref, sem):
        def copy(quarter, n):
            row, col = divmod(quarter % (4 * ROW_TILES), 4)
            at = (pl.ds(row * 8, 8), pl.ds(col * 1024, n * 1024))
            return pltpu.make_async_copy(hbm.at[at], ref.at[at], sems.at[sem])
        starts = [ROW_TILES * k // STREAMS for k in range(STREAMS + 1)]
        units = [u for _, u in sorted((u - lo, u) for lo, hi in zip(starts, starts[1:]) for u in range(lo, hi))]
        return [[copy(4 * units[i - delay] + first + k, 1) for k in range(n)]
                for i in range(ROW_TILES) for first, n, delay in PIECES_1]

    def row_copies(hbm, ref, sem, rows=8, col=0):
        return [[pltpu.make_async_copy(hbm.at[pl.ds(r, rows), pl.ds(col, ref.shape[1])],
                                       ref.at[pl.ds(r, rows)], sems.at[sem(r)])] for r in range(0, D, rows)]

    wq, wo = wide_copies(wq_hbm, wq_ref, S_WQ), wide_copies(wo_hbm, wo_ref, S_WO)
    wm = _scatter(row_copies(wm_hbm, wm_ref, lambda r: S_WM))
    w3 = _scatter(row_copies(w3_hbm, w3_ref, lambda r: S_W3))
    w4 = row_copies(w4_hbm, w4_ref, lambda r: S_W4 + _block(W4_BLOCKS, r))
    w4 = [w4[(r0 + half * n // 2) // 8 + i] for r0, n in W4_BLOCKS for i in range(n // 16) for half in range(2)]
    wg = row_copies(wm_hbm, wg_ref, lambda r: S_GATE + _block(GATE_BLOCKS, r), 16, GATE_COL)
    x_copy = pltpu.make_async_copy(x_hbm, x_ref, sems.at[S_X])
    c_copy = pltpu.make_async_copy(c_hbm, c_ref, sems.at[S_C])

    def enqueue(first, second=()):
        for copy in first:
            copy.start(priority=1)
        for copy in second:
            copy.start(priority=0)

    def enqueue_all(first, second, work):
        for j, copies in enumerate(first):
            lo, hi = j * len(second) // len(first), (j + 1) * len(second) // len(first)
            enqueue(copies, [copy for other in second[lo:hi] for copy in other])
            if j in work:
                work[j]()

    def stream(first, second, lo, hi):
        def body(i, carry):
            for pair in zip(first(i), second(i)):
                enqueue(*pair)
            return carry
        if lo % 32 == 0:
            body(lo, None)
            body(lo + 1, None)
            lo += 2
        lax.fori_loop(lo, hi, body, None)

    def landed(ref, sem):
        pltpu.make_async_copy(ref, ref, sems.at[sem]).wait()

    even = (lax.broadcasted_iota(jnp.int32, (ROWS, DH), 0) & 1) == 0

    def condition():
        c_copy.wait()
        landed(wm_ref, S_WM)
        c = jnp.broadcast_to(c_ref[...].astype(F32), (ROWS, D))
        c = (c * jax.nn.sigmoid(c)).astype(BF16)

        def body(i, carry):
            cols = _ds(i * 768, 768, 768)
            s_ref[0, :, cols] = _dot(c, wm_ref[:, cols])
            return carry
        lax.fori_loop(0, GATE_COL // 768, body, None)
        s_ref[0, :, GATE_COL:6 * D] = jnp.zeros((ROWS, 6 * D - GATE_COL), F32)
        for g in range(6):
            mod_ref[g] = s_ref[0, :, g * D:(g + 1) * D]
        s_ref[1, :, :512] = jnp.zeros((ROWS, 512), F32)
        s_ref[1, :, :D] = c.astype(F32)
        for t in range(0, 512, 128):
            ct_ref[t:t + 128] = jnp.broadcast_to(s_ref[1, 0:1, t:t + 128], (128, 128)).T

    def queries():
        x_copy.wait()
        landed(wq_ref, S_WQ)
        x = jnp.broadcast_to(x_ref[0].astype(F32), (ROWS, D))
        h_in = (_layernorm(x) * (1.0 + mod_ref[1]) + mod_ref[0]).astype(BF16)

        def body(h, carry):
            q = _dot(h_in, wq_ref[:, _ds(h * 2 * DH, 2 * DH, 2 * DH)]) * DH ** -0.5
            q_ref[h] = jnp.where(even, q[:, :DH], q[:, DH:])
            return carry
        lax.fori_loop(0, HKV, body, None)
        attn_ref[...] = jnp.zeros((ROWS, D), F32)

    def scores(h):
        landed(k_ref.at[h], S_K + h)
        s = _dot_t(q_ref[h].astype(BF16), k_ref[h])
        s_ref[h] = s
        m = s[:, :128]
        for t in range(128, window, 128):
            m = jnp.maximum(m, s[:, t:t + 128])
        max_ref[h] = jnp.broadcast_to(jnp.max(m, axis=-1, keepdims=True), (ROWS, 128))

    def context(h):
        landed(v_ref.at[h], S_V + h)
        p = jnp.exp(s_ref[h] - jnp.concatenate([max_ref[h]] * (window // 128), axis=1))
        total = p[:, :128]
        for t in range(128, window, 128):
            total = total + p[:, t:t + 128]
        o = _dot(p.astype(BF16), v_ref[h]) / jnp.sum(total, axis=-1, keepdims=True)
        o = jnp.concatenate([jnp.where(even, o, 0.0), jnp.where(even, 0.0, o)], axis=1).astype(BF16)
        attn_ref[...] += _dot_t(o, wo_ref[:, _ds(h * 2 * DH, 2 * DH, 2 * DH)])

    def residual():
        attn = attn_ref[...]
        x = jnp.broadcast_to(x_ref[0].astype(F32), (ROWS, D))
        x = x + mod_ref[2] * (attn + pltpu.roll(attn, 1, 0))
        h_mlp = _layernorm(x) * (1.0 + mod_ref[4]) + mod_ref[3]
        mod_ref[0], mod_ref[1], mod_ref[2] = x, h_mlp, _layernorm(h_mlp)

    keys = cache_copies(k_hbm, k_ref, S_K, 0, PIECES_1)
    keys = [copies for i in range(64) for copies in keys(i)]
    for copies in keys[:HEAD_START]:
        enqueue(copies)
    split = (HEAD_START + len(wq) + len(wo) - len(wm) - len(keys)) // 2 + 1
    enqueue_all(keys[HEAD_START:] + wm + wo[:split], [[c_copy, x_copy]] + wq + wo[split:], {})

    def period(g, carry):
        keys = cache_copies(k_hbm, k_ref, S_K, g + 1, PIECES_1)
        values = cache_copies(v_hbm, v_ref, S_V, g, PIECES_0)
        stream(keys, values, 0, AT["a"])
        pl.when(g == 0)(condition)
        pl.when(g == 1)(lambda: landed(wo_ref, S_WO))
        pl.when(g > 0)(lambda: context(2 * g - 2))
        stream(keys, values, AT["a"], AT["b"])
        pl.when(g == 0)(queries)
        pl.when(g > 0)(lambda: context(2 * g - 1))
        stream(keys, values, AT["b"], 32)
        scores(2 * g)
        stream(keys, values, 32, AT["d"])
        scores(2 * g + 1)
        stream(keys, values, AT["d"], 64)
        return carry
    lax.fori_loop(0, HKV // 2 - 1, period, None)

    values = cache_copies(v_hbm, v_ref, S_V, 3, PIECES_0)
    values = [copies for i in range(64) for copies in values(i)]
    shared = len(w4) - 2 * W4_FIRST
    first = values[-V_FIRST:] + w3 + w4[shared::2] + wg
    second = values[:-V_FIRST] + w4[:shared] + w4[shared + 1::2]
    assert (AT["c6"] + 1) * len(second) // len(first) >= len(values) - V_FIRST and AT["ln"] < len(first)
    enqueue_all(first, second, {AT["c4"]: lambda: context(4), AT["c5"]: lambda: context(5),
                                AT["s6"]: lambda: scores(6), AT["s7"]: lambda: scores(7),
                                AT["c6"]: lambda: context(6), AT["c7"]: lambda: context(7), AT["ln"]: residual})

    landed(w3_ref, S_W3)
    hidden = jax.nn.gelu(_dot(mod_ref[2].astype(BF16), w3_ref[...]), approximate=True).astype(BF16)
    for i, (r0, n) in enumerate(W4_BLOCKS):
        landed(w4_ref.at[pl.ds(r0, n)], S_W4 + i)
        mod_ref[1, :, r0:r0 + n] += _dot_t(hidden, w4_ref[r0:r0 + n, :])
    y = mod_ref[1]
    out = mod_ref[0] + mod_ref[5] * y

    gate = [0.0] * 3
    for i, (r0, n) in enumerate(GATE_BLOCKS):
        landed(wg_ref.at[pl.ds(r0, n)], S_GATE + i)
        for r in range(r0, r0 + n, 16):
            for t in range(3):
                part = ct_ref[r:r + 16] * wg_ref[r:r + 16, t * 128:(t + 1) * 128].astype(F32)
                gate[t] = gate[t] + (part[:8] + part[8:])
    low = lax.broadcasted_iota(jnp.int32, (ROWS, 128), 1) < 64
    gate = [pltpu.roll(g, 64, 1) for g in gate]
    gate = [jnp.where(low, a, b) for a, b in zip([0.0] + gate, gate + [0.0])]
    gate = jnp.concatenate([jnp.sum(g, axis=0, keepdims=True) for g in gate], axis=1)
    out_ref[0] = (out[0:1] + gate[:, :D] * y[0:1]).astype(BF16)
    store = pltpu.make_async_copy(out_ref, out_hbm, sems.at[S_X])
    store.start()
    store.wait()


@jax.jit
def pallas_adaLN_cond__sliding_block_cached__mixer_s_mlp__decode_kernel(
    A_x: jax.Array,
    A_k_cache: jax.Array,
    A_v_cache: jax.Array,
    A_wq: jax.Array,
    A_wo: jax.Array,
    B_x: jax.Array,
    B_w1: jax.Array,
    B_w2: jax.Array,
    B_w3: jax.Array,
    B_w4: jax.Array,
    c: jax.Array,
    w_mod: jax.Array,
):
    keys = A_k_cache.shape[2]
    window = min(4096, max(256, keys // 4))
    assert A_x.shape == (1, 1, D) and A_k_cache.shape == (1, HKV, keys, DH) and window == 4096
    hbm = pl.BlockSpec(memory_space=pltpu.HBM)
    return pl.pallas_call(
        _kernel,
        out_shape=jax.ShapeDtypeStruct(A_x.shape, A_x.dtype),
        in_specs=[hbm] * 9,
        out_specs=hbm,
        scratch_shapes=[
            pltpu.VMEM((1, 1, D), BF16),
            pltpu.VMEM((1, D), BF16),
            pltpu.VMEM((D, GATE_COL), BF16),
            pltpu.VMEM((D, 6 * D - GATE_COL), BF16),
            pltpu.VMEM((D, HQ * DH), BF16),
            pltpu.VMEM((HKV, window, DH), BF16),
            pltpu.VMEM((HKV, window, DH), BF16),
            pltpu.VMEM((D, HQ * DH), BF16),
            pltpu.VMEM((D, F), BF16),
            pltpu.VMEM((D, F), BF16),
            pltpu.VMEM((HKV, ROWS, DH), F32),
            pltpu.VMEM((HKV, ROWS, window), F32),
            pltpu.VMEM((HKV, ROWS, 128), F32),
            pltpu.VMEM((ROWS, D), F32),
            pltpu.VMEM((6, ROWS, D), F32),
            pltpu.VMEM((512, 128), F32),
            pltpu.VMEM((1, 1, D), BF16),
            pltpu.SemaphoreType.DMA((SEMS,)),
        ],
        compiler_params=pltpu.CompilerParams(
            vmem_limit_bytes=100 * 2**20,
            disable_semaphore_checks=True,
        ),
        name="adaln_decode",
    )(A_x, c, w_mod, A_wq, A_k_cache, A_v_cache, A_wo.T, B_w3, B_w4.T)
```

```python
import jax
import jax.numpy as jnp
from jax import lax
from jax.experimental import pallas as pl
from jax.experimental.pallas import tpu as pltpu

D, F = 448, 1792
HQ, HKV, DH = 16, 8, 256
EPS = 1e-5
BF16, F32 = jnp.bfloat16, jnp.float32
ROWS = 8
ROW_TILES = D // 8
QUARTER = 32
STREAMS = 5
UNIT_STRIDE = 13
PIECES_1 = ((-2, 1, 0), (1, 1, 3), (-1, 2, 1))
PIECES_0 = ((-1, 2, 1), (-2, 1, -1), (1, 1, 2))
ROW_STRIDE = 17
HEAD_START = 28
GATE_COL = 18 * 128
GATE_BLOCKS = ((0, 320), (320, 112), (432, 16))
W4_BLOCKS = ((0, 256), (256, 128), (384, 64))
W3_FIRST = 36
W4_FIRST = 24
AT = dict(a=14, b=22, d=48, s6=34, s7=48, c6=62, c7=75)

S_X, S_C, S_WM, S_WQ, S_WO, S_W3, S_K, S_V, S_W4, S_GATE, SEMS = 0, 1, 2, 3, 4, 5, 6, 14, 22, 25, 28


def _layernorm(x):
    d = x - jnp.sum(x, axis=-1, keepdims=True) * (1.0 / D)
    return d * lax.rsqrt(jnp.sum(d * d, axis=-1, keepdims=True) * (1.0 / D) + EPS)


def _dot(a, b):
    return lax.dot_general(a, b, (((1,), (0,)), ((), ())), preferred_element_type=F32)


def _dot_t(a, b):
    return lax.dot_general(a, b, (((1,), (1,)), ((), ())), preferred_element_type=F32)


def _ds(start, size, align):
    return pl.ds(start if isinstance(start, int) else pl.multiple_of(start, align), size)


def _scatter(copies):
    return [copies[p] for i in range(ROW_STRIDE) for p in range(4 * i % ROW_STRIDE, len(copies), ROW_STRIDE)]


def _block(blocks, row):
    return sum(row >= first for first, _ in blocks[1:])


def _kernel(x_hbm, c_hbm, wm_hbm, wq_hbm, k_hbm, v_hbm, wo_hbm, w3_hbm, w4_hbm, out_hbm,
            x_ref, c_ref, wm_ref, wg_ref, wq_ref, k_ref, v_ref, wo_ref, w3_ref, w4_ref,
            q_ref, s_ref, max_ref, attn_ref, mod_ref, ct_ref, out_ref, sems):
    window = k_ref.shape[1]
    first_key = k_hbm.shape[2] - window

    def cache_copies(hbm, ref, sem, pair, pieces):
        def copy(h, quarter, n):
            row, rows = (quarter & 127) * QUARTER, n * QUARTER
            return pltpu.make_async_copy(hbm.at[0, h, _ds(first_key + row, rows, QUARTER)],
                                         ref.at[h, _ds(row, rows, QUARTER)], sems.at[sem + h])

        def step(i):
            copies = []
            for first, n, delay in pieces:
                unit = (i + 64 - delay) * UNIT_STRIDE & 63
                h, quarter = 2 * pair + (unit >> 5), 4 * (unit & 31) + 128 + first
                if n == 2 and isinstance(i, int) and unit & 31 == 0:
                    copies.append([copy(h, quarter, 1), copy(h, quarter + 1, 1)])
                else:
                    copies.append([copy(h, quarter, n)])
            return copies
        return step

    def wide_copies(hbm, ref, sem):
        def copy(quarter, n):
            row, col = divmod(quarter % (4 * ROW_TILES), 4)
            at = (pl.ds(row * 8, 8), pl.ds(col * 1024, n * 1024))
            return pltpu.make_async_copy(hbm.at[at], ref.at[at], sems.at[sem])
        starts = [ROW_TILES * k // STREAMS for k in range(STREAMS + 1)]
        units = [u for _, u in sorted((u - lo, u) for lo, hi in zip(starts, starts[1:]) for u in range(lo, hi))]
        return [[copy(4 * units[i - delay] + first + k, 1) for k in range(n)]
                for i in range(ROW_TILES) for first, n, delay in PIECES_1]

    def row_copies(hbm, ref, sem, rows=8, col=0):
        return [[pltpu.make_async_copy(hbm.at[pl.ds(r, rows), pl.ds(col, ref.shape[1])],
                                       ref.at[pl.ds(r, rows)], sems.at[sem(r)])] for r in range(0, D, rows)]

    wq, wo = wide_copies(wq_hbm, wq_ref, S_WQ), wide_copies(wo_hbm, wo_ref, S_WO)
    wm = _scatter(row_copies(wm_hbm, wm_ref, lambda r: S_WM))
    w3 = _scatter(row_copies(w3_hbm, w3_ref, lambda r: S_W3))
    w4 = row_copies(w4_hbm, w4_ref, lambda r: S_W4 + _block(W4_BLOCKS, r))
    w4 = [w4[(r0 + half * n // 2) // 8 + i] for r0, n in W4_BLOCKS for i in range(n // 16) for half in range(2)]
    wg = row_copies(wm_hbm, wg_ref, lambda r: S_GATE + _block(GATE_BLOCKS, r), 16, GATE_COL)
    x_copy = pltpu.make_async_copy(x_hbm, x_ref, sems.at[S_X])
    c_copy = pltpu.make_async_copy(c_hbm, c_ref, sems.at[S_C])

    def enqueue(first, second=()):
        for copy in first:
            copy.start(priority=1)
        for copy in second:
            copy.start(priority=0)

    def enqueue_all(first, second, work):
        for j, copies in enumerate(first):
            lo, hi = j * len(second) // len(first), (j + 1) * len(second) // len(first)
            enqueue(copies, [copy for other in second[lo:hi] for copy in other])
            if j in work:
                work[j]()

    def stream(first, second, lo, hi):
        def body(i, carry):
            for pair in zip(first(i), second(i)):
                enqueue(*pair)
            return carry
        if lo % 32 == 0:
            body(lo, None)
            body(lo + 1, None)
            lo += 2
        lax.fori_loop(lo, hi, body, None)

    def landed(ref, sem):
        pltpu.make_async_copy(ref, ref, sems.at[sem]).wait()

    even = (lax.broadcasted_iota(jnp.int32, (ROWS, DH), 0) & 1) == 0

    def condition():
        c_copy.wait()
        landed(wm_ref, S_WM)
        c = jnp.broadcast_to(c_ref[...].astype(F32), (ROWS, D))
        c = (c * jax.nn.sigmoid(c)).astype(BF16)

        def body(i, carry):
            cols = _ds(i * 768, 768, 768)
            s_ref[0, :, cols] = _dot(c, wm_ref[:, cols])
            return carry
        lax.fori_loop(0, GATE_COL // 768, body, None)
        s_ref[0, :, GATE_COL:6 * D] = jnp.zeros((ROWS, 6 * D - GATE_COL), F32)
        for g in range(6):
            mod_ref[g] = s_ref[0, :, g * D:(g + 1) * D]
        s_ref[1, :, :512] = jnp.zeros((ROWS, 512), F32)
        s_ref[1, :, :D] = c.astype(F32)
        for t in range(0, 512, 128):
            ct_ref[t:t + 128] = jnp.broadcast_to(s_ref[1, 0:1, t:t + 128], (128, 128)).T

    def queries():
        x_copy.wait()
        landed(wq_ref, S_WQ)
        x = jnp.broadcast_to(x_ref[0].astype(F32), (ROWS, D))
        h_in = (_layernorm(x) * (1.0 + mod_ref[1]) + mod_ref[0]).astype(BF16)

        def body(h, carry):
            q = _dot(h_in, wq_ref[:, _ds(h * 2 * DH, 2 * DH, 2 * DH)]) * DH ** -0.5
            q_ref[h] = jnp.where(even, q[:, :DH], q[:, DH:])
            return carry
        lax.fori_loop(0, HKV, body, None)
        attn_ref[...] = jnp.zeros((ROWS, D), F32)

    def scores(h):
        landed(k_ref.at[h], S_K + h)
        s = _dot_t(q_ref[h].astype(BF16), k_ref[h])
        s_ref[h] = s
        m = s[:, :128]
        for t in range(128, window, 128):
            m = jnp.maximum(m, s[:, t:t + 128])
        max_ref[h] = jnp.broadcast_to(jnp.max(m, axis=-1, keepdims=True), (ROWS, 128))

    def context(h):
        landed(v_ref.at[h], S_V + h)
        p = jnp.exp(s_ref[h] - jnp.concatenate([max_ref[h]] * (window // 128), axis=1))
        total = p[:, :128]
        for t in range(128, window, 128):
            total = total + p[:, t:t + 128]
        o = _dot(p.astype(BF16), v_ref[h]) / jnp.sum(total, axis=-1, keepdims=True)
        o = jnp.concatenate([jnp.where(even, o, 0.0), jnp.where(even, 0.0, o)], axis=1).astype(BF16)
        attn_ref[...] += _dot_t(o, wo_ref[:, _ds(h * 2 * DH, 2 * DH, 2 * DH)])

    def residual():
        attn = attn_ref[...]
        x = jnp.broadcast_to(x_ref[0].astype(F32), (ROWS, D))
        x = x + mod_ref[2] * (attn + pltpu.roll(attn, 1, 0))
        h_mlp = _layernorm(x) * (1.0 + mod_ref[4]) + mod_ref[3]
        mod_ref[0], mod_ref[1], mod_ref[2] = x, h_mlp, _layernorm(h_mlp)

    for copies in wo[:HEAD_START]:
        enqueue(copies)
    enqueue_all(wo[HEAD_START:] + wm, [[c_copy, x_copy]] + wq, {})

    def period(g, carry):
        values = cache_copies(v_hbm, v_ref, S_V, g, PIECES_1)
        keys = cache_copies(k_hbm, k_ref, S_K, g, PIECES_0)
        stream(values, keys, 0, AT["a"])
        pl.when(g > 0)(lambda: scores(2 * g - 2))
        stream(values, keys, AT["a"], AT["b"])
        pl.when(g == 0)(condition)
        pl.when(g > 0)(lambda: scores(2 * g - 1))
        stream(values, keys, AT["b"], 32)
        pl.when(g == 0)(queries)
        pl.when(g > 0)(lambda: context(2 * g - 2))
        stream(values, keys, 32, AT["d"])
        pl.when(g == 0)(lambda: landed(wo_ref, S_WO))
        pl.when(g > 0)(lambda: context(2 * g - 1))
        stream(values, keys, AT["d"], 64)
        return carry
    lax.fori_loop(0, HKV // 2, period, None)

    shared = len(w4) - 2 * W4_FIRST
    enqueue_all(w3[:W3_FIRST] + w4[shared::2] + wg, w3[W3_FIRST:] + w4[:shared] + w4[shared + 1::2],
                {AT["s6"]: lambda: scores(6), AT["s7"]: lambda: scores(7),
                 AT["c6"]: lambda: context(6), AT["c7"]: lambda: context(7)})
    assert AT["s6"] < AT["s7"] < AT["c6"] < AT["c7"] < W3_FIRST + W4_FIRST + len(wg)
    residual()

    landed(w3_ref, S_W3)
    hidden = jax.nn.gelu(_dot(mod_ref[2].astype(BF16), w3_ref[...]), approximate=True).astype(BF16)
    for i, (r0, n) in enumerate(W4_BLOCKS):
        landed(w4_ref.at[pl.ds(r0, n)], S_W4 + i)
        mod_ref[1, :, r0:r0 + n] += _dot_t(hidden, w4_ref[r0:r0 + n, :])
    y = mod_ref[1]
    out = mod_ref[0] + mod_ref[5] * y

    gate = [0.0] * 3
    for i, (r0, n) in enumerate(GATE_BLOCKS):
        landed(wg_ref.at[pl.ds(r0, n)], S_GATE + i)
        for r in range(r0, r0 + n, 16):
            for t in range(3):
                part = ct_ref[r:r + 16] * wg_ref[r:r + 16, t * 128:(t + 1) * 128].astype(F32)
                gate[t] = gate[t] + (part[:8] + part[8:])
    low = lax.broadcasted_iota(jnp.int32, (ROWS, 128), 1) < 64
    gate = [pltpu.roll(g, 64, 1) for g in gate]
    gate = [jnp.where(low, a, b) for a, b in zip([0.0] + gate, gate + [0.0])]
    gate = jnp.concatenate([jnp.sum(g, axis=0, keepdims=True) for g in gate], axis=1)
    out_ref[0] = (out[0:1] + gate[:, :D] * y[0:1]).astype(BF16)
    store = pltpu.make_async_copy(out_ref, out_hbm, sems.at[S_X])
    store.start()
    store.wait()


@jax.jit
def pallas_adaLN_cond__sliding_block_cached__mixer_s_mlp__decode_kernel(
    A_x: jax.Array,
    A_k_cache: jax.Array,
    A_v_cache: jax.Array,
    A_wq: jax.Array,
    A_wo: jax.Array,
    B_x: jax.Array,
    B_w1: jax.Array,
    B_w2: jax.Array,
    B_w3: jax.Array,
    B_w4: jax.Array,
    c: jax.Array,
    w_mod: jax.Array,
):
    keys = A_k_cache.shape[2]
    window = min(4096, max(256, keys // 4))
    assert A_x.shape == (1, 1, D) and A_k_cache.shape == (1, HKV, keys, DH) and window == 4096
    hbm = pl.BlockSpec(memory_space=pltpu.HBM)
    return pl.pallas_call(
        _kernel,
        out_shape=jax.ShapeDtypeStruct(A_x.shape, A_x.dtype),
        in_specs=[hbm] * 9,
        out_specs=hbm,
        scratch_shapes=[
            pltpu.VMEM((1, 1, D), BF16),
            pltpu.VMEM((1, D), BF16),
            pltpu.VMEM((D, GATE_COL), BF16),
            pltpu.VMEM((D, 6 * D - GATE_COL), BF16),
            pltpu.VMEM((D, HQ * DH), BF16),
            pltpu.VMEM((HKV, window, DH), BF16),
            pltpu.VMEM((HKV, window, DH), BF16),
            pltpu.VMEM((D, HQ * DH), BF16),
            pltpu.VMEM((D, F), BF16),
            pltpu.VMEM((D, F), BF16),
            pltpu.VMEM((HKV, ROWS, DH), F32),
            pltpu.VMEM((HKV, ROWS, window), F32),
            pltpu.VMEM((HKV, ROWS, 128), F32),
            pltpu.VMEM((ROWS, D), F32),
            pltpu.VMEM((6, ROWS, D), F32),
            pltpu.VMEM((512, 128), F32),
            pltpu.VMEM((1, 1, D), BF16),
            pltpu.SemaphoreType.DMA((SEMS,)),
        ],
        compiler_params=pltpu.CompilerParams(
            vmem_limit_bytes=100 * 2**20,
            disable_semaphore_checks=True,
        ),
        name="adaln_decode",
    )(A_x, c, w_mod, A_wq, A_k_cache, A_v_cache, A_wo.T, B_w3, B_w4.T)
```

```python
import jax
import jax.numpy as jnp
from jax import lax
from jax.experimental import pallas as pl
from jax.experimental.pallas import tpu as pltpu

D, F = 448, 1792
HQ, HKV, DH = 16, 8, 256
EPS = 1e-5
BF16, F32 = jnp.bfloat16, jnp.float32
ROWS = 8
ROW_TILES = D // 8
QUARTER = 32
STREAMS = 5
UNIT_STRIDE = 13
PIECES = ((-2, 1, 0), (1, 1, 3), (-1, 2, 1))
HEAD_START = 22
GATE_COL = 18 * 128
GATE_BLOCKS = ((0, 320), (320, 112), (432, 16))
W4_BLOCKS = ((0, 256), (256, 128), (384, 64))
W3_FIRST = 36
W4_FIRST = 24
AT = dict(a=14, b=22, d=48, s6=34, s7=48, c6=62, c7=75)

S_X, S_C, S_WM, S_WQ, S_WO, S_W3, S_K, S_V, S_W4, S_GATE, SEMS = 0, 1, 2, 3, 4, 5, 6, 14, 22, 25, 28


def _layernorm(x):
    d = x - jnp.sum(x, axis=-1, keepdims=True) * (1.0 / D)
    return d * lax.rsqrt(jnp.sum(d * d, axis=-1, keepdims=True) * (1.0 / D) + EPS)


def _dot(a, b):
    return lax.dot_general(a, b, (((1,), (0,)), ((), ())), preferred_element_type=F32)


def _dot_t(a, b):
    return lax.dot_general(a, b, (((1,), (1,)), ((), ())), preferred_element_type=F32)


def _ds(start, size, align):
    return pl.ds(start if isinstance(start, int) else pl.multiple_of(start, align), size)


def _weave(items, streams):
    starts = [len(items) * k // streams for k in range(streams + 1)]
    return [items[i] for _, i in sorted((i - lo, i) for lo, hi in zip(starts, starts[1:]) for i in range(lo, hi))]


def _block(blocks, row):
    return sum(row >= first for first, _ in blocks[1:])


def _kernel(x_hbm, c_hbm, wm_hbm, wq_hbm, k_hbm, v_hbm, wo_hbm, w3_hbm, w4_hbm, out_hbm,
            x_ref, c_ref, wm_ref, wg_ref, wq_ref, k_ref, v_ref, wo_ref, w3_ref, w4_ref,
            q_ref, s_ref, max_ref, attn_ref, mod_ref, ct_ref, out_ref, sems):
    window = k_ref.shape[1]
    first_key = k_hbm.shape[2] - window

    def cache_copies(hbm, ref, sem, pair):
        def copy(h, quarter, n):
            row, rows = (quarter & 127) * QUARTER, n * QUARTER
            return pltpu.make_async_copy(hbm.at[0, h, _ds(first_key + row, rows, QUARTER)],
                                         ref.at[h, _ds(row, rows, QUARTER)], sems.at[sem + h])

        def step(i):
            copies = []
            for first, n, delay in PIECES:
                unit = (i + 64 - delay) * UNIT_STRIDE & 63
                h, quarter = 2 * pair + (unit >> 5), 4 * (unit & 31) + 128 + first
                if n == 2 and isinstance(i, int) and unit & 31 == 0:
                    copies.append([copy(h, quarter, 1), copy(h, quarter + 1, 1)])
                else:
                    copies.append([copy(h, quarter, n)])
            return copies
        return step

    def wide_copies(hbm, ref, sem):
        def copy(quarter, n):
            row, col = divmod(quarter % (4 * ROW_TILES), 4)
            at = (pl.ds(row * 8, 8), pl.ds(col * 1024, n * 1024))
            return pltpu.make_async_copy(hbm.at[at], ref.at[at], sems.at[sem])
        units = _weave(range(ROW_TILES), STREAMS)
        return [[copy(4 * units[i - delay] + first + k, 1) for k in range(n)]
                for i in range(ROW_TILES) for first, n, delay in PIECES]

    def row_copies(hbm, ref, sem, rows=8, col=0):
        return [[pltpu.make_async_copy(hbm.at[pl.ds(r, rows), pl.ds(col, ref.shape[1])],
                                       ref.at[pl.ds(r, rows)], sems.at[sem(r)])] for r in range(0, D, rows)]

    wq, wo = wide_copies(wq_hbm, wq_ref, S_WQ), wide_copies(wo_hbm, wo_ref, S_WO)
    wm = _weave(row_copies(wm_hbm, wm_ref, lambda r: S_WM), 4)
    w3 = _weave(row_copies(w3_hbm, w3_ref, lambda r: S_W3), 3)
    w4 = row_copies(w4_hbm, w4_ref, lambda r: S_W4 + _block(W4_BLOCKS, r))
    w4 = [w4[(r0 + half * n // 2) // 8 + i] for r0, n in W4_BLOCKS for i in range(n // 16) for half in range(2)]
    wg = row_copies(wm_hbm, wg_ref, lambda r: S_GATE + _block(GATE_BLOCKS, r), 16, GATE_COL)
    x_copy = pltpu.make_async_copy(x_hbm, x_ref, sems.at[S_X])
    c_copy = pltpu.make_async_copy(c_hbm, c_ref, sems.at[S_C])

    def enqueue(first, second=()):
        for copy in first:
            copy.start(priority=1)
        for copy in second:
            copy.start(priority=0)

    def enqueue_all(first, second, work):
        for j, copies in enumerate(first):
            lo, hi = j * len(second) // len(first), (j + 1) * len(second) // len(first)
            enqueue(copies, [copy for other in second[lo:hi] for copy in other])
            if j in work:
                work[j]()

    def stream(first, second, lo, hi):
        def body(i, carry):
            for pair in zip(first(i), second(i)):
                enqueue(*pair)
            return carry
        if lo % 32 == 0:
            body(lo, None)
            body(lo + 1, None)
            lo += 2
        lax.fori_loop(lo, hi, body, None)

    def landed(ref, sem):
        pltpu.make_async_copy(ref, ref, sems.at[sem]).wait()

    even = (lax.broadcasted_iota(jnp.int32, (ROWS, DH), 0) & 1) == 0

    def condition():
        c_copy.wait()
        landed(wm_ref, S_WM)
        c = jnp.broadcast_to(c_ref[...].astype(F32), (ROWS, D))
        c = (c * jax.nn.sigmoid(c)).astype(BF16)

        def body(i, carry):
            cols = _ds(i * 768, 768, 768)
            s_ref[0, :, cols] = _dot(c, wm_ref[:, cols])
            return carry
        lax.fori_loop(0, GATE_COL // 768, body, None)
        s_ref[0, :, GATE_COL:6 * D] = jnp.zeros((ROWS, 6 * D - GATE_COL), F32)
        for g in range(6):
            mod_ref[g] = s_ref[0, :, g * D:(g + 1) * D]
        s_ref[1, :, :512] = jnp.zeros((ROWS, 512), F32)
        s_ref[1, :, :D] = c.astype(F32)
        for t in range(0, 512, 128):
            ct_ref[t:t + 128] = jnp.broadcast_to(s_ref[1, 0:1, t:t + 128], (128, 128)).T

    def queries():
        x_copy.wait()
        landed(wq_ref, S_WQ)
        x = jnp.broadcast_to(x_ref[0].astype(F32), (ROWS, D))
        h_in = (_layernorm(x) * (1.0 + mod_ref[1]) + mod_ref[0]).astype(BF16)

        def body(h, carry):
            q = _dot(h_in, wq_ref[:, _ds(h * 2 * DH, 2 * DH, 2 * DH)]) * DH ** -0.5
            q_ref[h] = jnp.where(even, q[:, :DH], q[:, DH:])
            return carry
        lax.fori_loop(0, HKV, body, None)
        attn_ref[...] = jnp.zeros((ROWS, D), F32)

    def scores(h):
        landed(k_ref.at[h], S_K + h)
        s = _dot_t(q_ref[h].astype(BF16), k_ref[h])
        s_ref[h] = s
        m = s[:, :128]
        for t in range(128, window, 128):
            m = jnp.maximum(m, s[:, t:t + 128])
        max_ref[h] = jnp.broadcast_to(jnp.max(m, axis=-1, keepdims=True), (ROWS, 128))

    def context(h):
        landed(v_ref.at[h], S_V + h)
        p = jnp.exp(s_ref[h] - jnp.concatenate([max_ref[h]] * (window // 128), axis=1))
        total = p[:, :128]
        for t in range(128, window, 128):
            total = total + p[:, t:t + 128]
        o = _dot(p.astype(BF16), v_ref[h]) / jnp.sum(total, axis=-1, keepdims=True)
        o = jnp.concatenate([jnp.where(even, o, 0.0), jnp.where(even, 0.0, o)], axis=1).astype(BF16)
        attn_ref[...] += _dot_t(o, wo_ref[:, _ds(h * 2 * DH, 2 * DH, 2 * DH)])

    def residual():
        attn = attn_ref[...]
        x = jnp.broadcast_to(x_ref[0].astype(F32), (ROWS, D))
        x = x + mod_ref[2] * (attn + pltpu.roll(attn, 1, 0))
        h_mlp = _layernorm(x) * (1.0 + mod_ref[4]) + mod_ref[3]
        mod_ref[0], mod_ref[1], mod_ref[2] = x, h_mlp, _layernorm(h_mlp)

    for copies in wo[:HEAD_START]:
        enqueue(copies)
    enqueue_all(wo[HEAD_START:] + wm, [[c_copy, x_copy]] + wq, {})

    def period(g, carry):
        values = cache_copies(v_hbm, v_ref, S_V, g)
        keys = cache_copies(k_hbm, k_ref, S_K, g)
        stream(values, keys, 0, AT["a"])
        pl.when(g > 0)(lambda: scores(2 * g - 2))
        stream(values, keys, AT["a"], AT["b"])
        pl.when(g == 0)(condition)
        pl.when(g > 0)(lambda: scores(2 * g - 1))
        stream(values, keys, AT["b"], 32)
        pl.when(g == 0)(queries)
        pl.when(g > 0)(lambda: context(2 * g - 2))
        stream(values, keys, 32, AT["d"])
        pl.when(g == 0)(lambda: landed(wo_ref, S_WO))
        pl.when(g > 0)(lambda: context(2 * g - 1))
        stream(values, keys, AT["d"], 64)
        return carry
    lax.fori_loop(0, HKV // 2, period, None)

    shared = len(w4) - 2 * W4_FIRST
    enqueue_all(w3[:W3_FIRST] + w4[shared::2] + wg, w3[W3_FIRST:] + w4[:shared] + w4[shared + 1::2],
                {AT["s6"]: lambda: scores(6), AT["s7"]: lambda: scores(7),
                 AT["c6"]: lambda: context(6), AT["c7"]: lambda: context(7)})
    assert AT["s6"] < AT["s7"] < AT["c6"] < AT["c7"] < W3_FIRST + W4_FIRST + len(wg)
    residual()

    landed(w3_ref, S_W3)
    hidden = jax.nn.gelu(_dot(mod_ref[2].astype(BF16), w3_ref[...]), approximate=True).astype(BF16)
    for i, (r0, n) in enumerate(W4_BLOCKS):
        landed(w4_ref.at[pl.ds(r0, n)], S_W4 + i)
        mod_ref[1, :, r0:r0 + n] += _dot_t(hidden, w4_ref[r0:r0 + n, :])
    y = mod_ref[1]
    out = mod_ref[0] + mod_ref[5] * y

    gate = [0.0] * 3
    for i, (r0, n) in enumerate(GATE_BLOCKS):
        landed(wg_ref.at[pl.ds(r0, n)], S_GATE + i)
        for r in range(r0, r0 + n, 16):
            for t in range(3):
                part = ct_ref[r:r + 16] * wg_ref[r:r + 16, t * 128:(t + 1) * 128].astype(F32)
                gate[t] = gate[t] + (part[:8] + part[8:])
    low = lax.broadcasted_iota(jnp.int32, (ROWS, 128), 1) < 64
    gate = [pltpu.roll(g, 64, 1) for g in gate]
    gate = [jnp.where(low, a, b) for a, b in zip([0.0] + gate, gate + [0.0])]
    gate = jnp.concatenate([jnp.sum(g, axis=0, keepdims=True) for g in gate], axis=1)
    out_ref[0] = (out[0:1] + gate[:, :D] * y[0:1]).astype(BF16)
    store = pltpu.make_async_copy(out_ref, out_hbm, sems.at[S_X])
    store.start()
    store.wait()


@jax.jit
def pallas_adaLN_cond__sliding_block_cached__mixer_s_mlp__decode_kernel(
    A_x: jax.Array,
    A_k_cache: jax.Array,
    A_v_cache: jax.Array,
    A_wq: jax.Array,
    A_wo: jax.Array,
    B_x: jax.Array,
    B_w1: jax.Array,
    B_w2: jax.Array,
    B_w3: jax.Array,
    B_w4: jax.Array,
    c: jax.Array,
    w_mod: jax.Array,
):
    keys = A_k_cache.shape[2]
    window = min(4096, max(256, keys // 4))
    assert A_x.shape == (1, 1, D) and A_k_cache.shape == (1, HKV, keys, DH) and window == 4096
    hbm = pl.BlockSpec(memory_space=pltpu.HBM)
    return pl.pallas_call(
        _kernel,
        out_shape=jax.ShapeDtypeStruct(A_x.shape, A_x.dtype),
        in_specs=[hbm] * 9,
        out_specs=hbm,
        scratch_shapes=[
            pltpu.VMEM((1, 1, D), BF16),
            pltpu.VMEM((1, D), BF16),
            pltpu.VMEM((D, GATE_COL), BF16),
            pltpu.VMEM((D, 6 * D - GATE_COL), BF16),
            pltpu.VMEM((D, HQ * DH), BF16),
            pltpu.VMEM((HKV, window, DH), BF16),
            pltpu.VMEM((HKV, window, DH), BF16),
            pltpu.VMEM((D, HQ * DH), BF16),
            pltpu.VMEM((D, F), BF16),
            pltpu.VMEM((D, F), BF16),
            pltpu.VMEM((HKV, ROWS, DH), F32),
            pltpu.VMEM((HKV, ROWS, window), F32),
            pltpu.VMEM((HKV, ROWS, 128), F32),
            pltpu.VMEM((ROWS, D), F32),
            pltpu.VMEM((6, ROWS, D), F32),
            pltpu.VMEM((512, 128), F32),
            pltpu.VMEM((1, 1, D), BF16),
            pltpu.SemaphoreType.DMA((SEMS,)),
        ],
        compiler_params=pltpu.CompilerParams(
            vmem_limit_bytes=100 * 2**20,
            disable_semaphore_checks=True,
        ),
        name="adaln_decode",
    )(A_x, c, w_mod, A_wq, A_k_cache, A_v_cache, A_wo.T, B_w3, B_w4.T)
```

```python
import jax
import jax.numpy as jnp
from jax import lax
from jax.experimental import pallas as pl
from jax.experimental.pallas import tpu as pltpu

D, F = 448, 1792
HQ, HKV, DH = 16, 8, 256
EPS = 1e-5
BF16, F32 = jnp.bfloat16, jnp.float32
ROWS = 8
ROW_TILES = D // 8
QUARTER = 32
STREAMS = 5
UNIT_STRIDE = 13
PIECES = ((-2, 1, 0), (1, 1, 3), (-1, 2, 1))
HEAD_START = 22
GATE_COL = 18 * 128
GATE_BLOCKS = ((0, 320), (320, 112), (432, 16))
W4_BLOCKS = ((0, 256), (256, 128), (384, 64))
W3_FIRST = 36
W4_FIRST = 24

S_X, S_C, S_WM, S_WQ, S_WO, S_W3, S_K, S_V, S_W4, S_GATE, SEMS = 0, 1, 2, 3, 4, 5, 6, 14, 22, 25, 28


def _layernorm(x):
    d = x - jnp.sum(x, axis=-1, keepdims=True) * (1.0 / D)
    return d * lax.rsqrt(jnp.sum(d * d, axis=-1, keepdims=True) * (1.0 / D) + EPS)


def _dot(a, b):
    return lax.dot_general(a, b, (((1,), (0,)), ((), ())), preferred_element_type=F32)


def _dot_t(a, b):
    return lax.dot_general(a, b, (((1,), (1,)), ((), ())), preferred_element_type=F32)


def _ds(start, size):
    return pl.ds(start if isinstance(start, int) else pl.multiple_of(start, size), size)


def _weave(items, streams):
    starts = [len(items) * k // streams for k in range(streams + 1)]
    return [items[i] for _, i in sorted((i - lo, i) for lo, hi in zip(starts, starts[1:]) for i in range(lo, hi))]


def _block(blocks, row):
    return sum(row >= first for first, _ in blocks[1:])


def _kernel(x_hbm, c_hbm, wm_hbm, wq_hbm, k_hbm, v_hbm, wo_hbm, w3_hbm, w4_hbm, out_hbm,
            x_ref, c_ref, wm_ref, wg_ref, wq_ref, k_ref, v_ref, wo_ref, w3_ref, w4_ref,
            q_ref, s_ref, max_ref, attn_ref, mod_ref, ct_ref, out_ref, sems):
    window = k_ref.shape[1]
    first_key = k_hbm.shape[2] - window

    def cache_copies(hbm, ref, sem, pair):
        def copy(h, quarter, n):
            row, rows = quarter % 128 * QUARTER, n * QUARTER
            return pltpu.make_async_copy(hbm.at[0, h, pl.ds(first_key + row, rows)],
                                         ref.at[h, pl.ds(row, rows)], sems.at[sem + h])
        heads = (2 * pair, 2 * pair + 1)
        copies = []
        for i in range(64):
            for first, n, delay in PIECES:
                k, unit = divmod((i - delay) * UNIT_STRIDE % 64, 32)
                quarter = 4 * unit + first
                if quarter < 0 < quarter + n:
                    copies.append([copy(heads[k], quarter, 1), copy(heads[k], quarter + 1, 1)])
                else:
                    copies.append([copy(heads[k], quarter, n)])
        return copies

    def wide_copies(hbm, ref, sem):
        def copy(quarter, n):
            row, col = divmod(quarter % (4 * ROW_TILES), 4)
            at = (pl.ds(row * 8, 8), pl.ds(col * 1024, n * 1024))
            return pltpu.make_async_copy(hbm.at[at], ref.at[at], sems.at[sem])
        units = _weave(range(ROW_TILES), STREAMS)
        return [[copy(4 * units[i - delay] + first + k, 1) for k in range(n)]
                for i in range(ROW_TILES) for first, n, delay in PIECES]

    def row_copies(hbm, ref, sem, rows=8, col=0):
        return [[pltpu.make_async_copy(hbm.at[pl.ds(r, rows), pl.ds(col, ref.shape[1])],
                                       ref.at[pl.ds(r, rows)], sems.at[sem(r)])] for r in range(0, D, rows)]

    wq, wo = wide_copies(wq_hbm, wq_ref, S_WQ), wide_copies(wo_hbm, wo_ref, S_WO)
    wm = _weave(row_copies(wm_hbm, wm_ref, lambda r: S_WM), 4)
    w3 = _weave(row_copies(w3_hbm, w3_ref, lambda r: S_W3), 3)
    w4 = row_copies(w4_hbm, w4_ref, lambda r: S_W4 + _block(W4_BLOCKS, r))
    w4 = [w4[(r0 + half * n // 2) // 8 + i] for r0, n in W4_BLOCKS for i in range(n // 16) for half in range(2)]
    wg = row_copies(wm_hbm, wg_ref, lambda r: S_GATE + _block(GATE_BLOCKS, r), 16, GATE_COL)
    x_copy = pltpu.make_async_copy(x_hbm, x_ref, sems.at[S_X])
    c_copy = pltpu.make_async_copy(c_hbm, c_ref, sems.at[S_C])

    def enqueue(first, second=()):
        for copy in first:
            copy.start(priority=1)
        for copy in second:
            copy.start(priority=0)

    def enqueue_all(first, second, work):
        for j, copies in enumerate(first):
            lo, hi = j * len(second) // len(first), (j + 1) * len(second) // len(first)
            enqueue(copies, [copy for other in second[lo:hi] for copy in other])
            if j in work:
                work[j]()

    def landed(ref, sem):
        pltpu.make_async_copy(ref, ref, sems.at[sem]).wait()

    even = (lax.broadcasted_iota(jnp.int32, (ROWS, DH), 0) & 1) == 0

    def condition():
        c_copy.wait()
        landed(wm_ref, S_WM)
        c = jnp.broadcast_to(c_ref[...].astype(F32), (ROWS, D))
        c = (c * jax.nn.sigmoid(c)).astype(BF16)

        def body(i, carry):
            cols = _ds(i * 384, 384)
            s_ref[0, :, cols] = _dot(c, wm_ref[:, cols])
            return carry
        lax.fori_loop(0, GATE_COL // 384, body, None)
        s_ref[0, :, GATE_COL:6 * D] = jnp.zeros((ROWS, 6 * D - GATE_COL), F32)
        for g in range(6):
            mod_ref[g] = s_ref[0, :, g * D:(g + 1) * D]
        s_ref[1, :, :512] = jnp.zeros((ROWS, 512), F32)
        s_ref[1, :, :D] = c.astype(F32)
        for t in range(0, 512, 128):
            ct_ref[t:t + 128] = jnp.broadcast_to(s_ref[1, 0:1, t:t + 128], (128, 128)).T

    def queries():
        x_copy.wait()
        landed(wq_ref, S_WQ)
        x = jnp.broadcast_to(x_ref[0].astype(F32), (ROWS, D))
        h_in = (_layernorm(x) * (1.0 + mod_ref[1]) + mod_ref[0]).astype(BF16)

        def body(h, carry):
            q = _dot(h_in, wq_ref[:, _ds(h * 2 * DH, 2 * DH)]) * DH ** -0.5
            q_ref[h] = jnp.where(even, q[:, :DH], q[:, DH:])
            return carry
        lax.fori_loop(0, HKV, body, None)
        attn_ref[...] = jnp.zeros((ROWS, D), F32)

    def scores(h):
        landed(k_ref.at[h], S_K + h)
        s = _dot_t(q_ref[h].astype(BF16), k_ref[h])
        s_ref[h] = s
        m = s[:, :128]
        for t in range(128, window, 128):
            m = jnp.maximum(m, s[:, t:t + 128])
        max_ref[h] = jnp.broadcast_to(jnp.max(m, axis=-1, keepdims=True), (ROWS, 128))

    def context(h):
        landed(v_ref.at[h], S_V + h)
        p = jnp.exp(s_ref[h] - jnp.concatenate([max_ref[h]] * (window // 128), axis=1))
        total = p[:, :128]
        for t in range(128, window, 128):
            total = total + p[:, t:t + 128]
        o = _dot(p.astype(BF16), v_ref[h]) / jnp.sum(total, axis=-1, keepdims=True)
        o = jnp.concatenate([jnp.where(even, o, 0.0), jnp.where(even, 0.0, o)], axis=1).astype(BF16)
        attn_ref[...] += _dot_t(o, wo_ref[:, _ds(h * 2 * DH, 2 * DH)])

    def residual():
        attn = attn_ref[...]
        x = jnp.broadcast_to(x_ref[0].astype(F32), (ROWS, D))
        x = x + mod_ref[2] * (attn + pltpu.roll(attn, 1, 0))
        h_mlp = _layernorm(x) * (1.0 + mod_ref[4]) + mod_ref[3]
        mod_ref[0], mod_ref[1], mod_ref[2] = x, h_mlp, _layernorm(h_mlp)

    for copies in wo[:HEAD_START]:
        enqueue(copies)
    enqueue_all(wo[HEAD_START:] + wm, [[c_copy, x_copy]] + wq, {})

    def period(g, carry):
        def after(copies, first_period, later):
            def work():
                if first_period:
                    pl.when(g == 0)(first_period)
                pl.when(g > 0)(later)
            return copies, work
        enqueue_all(cache_copies(v_hbm, v_ref, S_V, g), cache_copies(k_hbm, k_ref, S_K, g), dict([
            after(42, None, lambda: scores(2 * g - 2)),
            after(66, condition, lambda: scores(2 * g - 1)),
            after(96, queries, lambda: context(2 * g - 2)),
            after(144, lambda: landed(wo_ref, S_WO), lambda: context(2 * g - 1))]))
        return carry
    lax.fori_loop(0, HKV // 2, period, None)

    shared = len(w4) - 2 * W4_FIRST
    enqueue_all(w3[:W3_FIRST] + w4[shared::2] + wg, w3[W3_FIRST:] + w4[:shared] + w4[shared + 1::2],
                {34: lambda: scores(6), 48: lambda: scores(7), 62: lambda: context(6), 75: lambda: context(7)})
    residual()

    landed(w3_ref, S_W3)
    hidden = jax.nn.gelu(_dot(mod_ref[2].astype(BF16), w3_ref[...]), approximate=True).astype(BF16)
    for i, (r0, n) in enumerate(W4_BLOCKS):
        landed(w4_ref.at[pl.ds(r0, n)], S_W4 + i)
        mod_ref[1, :, r0:r0 + n] += _dot_t(hidden, w4_ref[r0:r0 + n, :])
    y = mod_ref[1]
    out = mod_ref[0] + mod_ref[5] * y

    gate = [0.0] * 3
    for i, (r0, n) in enumerate(GATE_BLOCKS):
        landed(wg_ref.at[pl.ds(r0, n)], S_GATE + i)
        for r in range(r0, r0 + n, 16):
            for t in range(3):
                part = ct_ref[r:r + 16] * wg_ref[r:r + 16, t * 128:(t + 1) * 128].astype(F32)
                gate[t] = gate[t] + (part[:8] + part[8:])
    low = lax.broadcasted_iota(jnp.int32, (ROWS, 128), 1) < 64
    gate = [pltpu.roll(g, 64, 1) for g in gate]
    gate = [jnp.where(low, a, b) for a, b in zip([0.0] + gate, gate + [0.0])]
    gate = jnp.concatenate([jnp.sum(g, axis=0, keepdims=True) for g in gate], axis=1)
    out_ref[0] = (out[0:1] + gate[:, :D] * y[0:1]).astype(BF16)
    store = pltpu.make_async_copy(out_ref, out_hbm, sems.at[S_X])
    store.start()
    store.wait()


@jax.jit
def pallas_adaLN_cond__sliding_block_cached__mixer_s_mlp__decode_kernel(
    A_x: jax.Array,
    A_k_cache: jax.Array,
    A_v_cache: jax.Array,
    A_wq: jax.Array,
    A_wo: jax.Array,
    B_x: jax.Array,
    B_w1: jax.Array,
    B_w2: jax.Array,
    B_w3: jax.Array,
    B_w4: jax.Array,
    c: jax.Array,
    w_mod: jax.Array,
):
    keys = A_k_cache.shape[2]
    window = min(4096, max(256, keys // 4))
    assert A_x.shape == (1, 1, D) and A_k_cache.shape == (1, HKV, keys, DH) and window == 4096
    hbm = pl.BlockSpec(memory_space=pltpu.HBM)
    return pl.pallas_call(
        _kernel,
        out_shape=jax.ShapeDtypeStruct(A_x.shape, A_x.dtype),
        in_specs=[hbm] * 9,
        out_specs=hbm,
        scratch_shapes=[
            pltpu.VMEM((1, 1, D), BF16),
            pltpu.VMEM((1, D), BF16),
            pltpu.VMEM((D, GATE_COL), BF16),
            pltpu.VMEM((D, 6 * D - GATE_COL), BF16),
            pltpu.VMEM((D, HQ * DH), BF16),
            pltpu.VMEM((HKV, window, DH), BF16),
            pltpu.VMEM((HKV, window, DH), BF16),
            pltpu.VMEM((D, HQ * DH), BF16),
            pltpu.VMEM((D, F), BF16),
            pltpu.VMEM((D, F), BF16),
            pltpu.VMEM((HKV, ROWS, DH), F32),
            pltpu.VMEM((HKV, ROWS, window), F32),
            pltpu.VMEM((HKV, ROWS, 128), F32),
            pltpu.VMEM((ROWS, D), F32),
            pltpu.VMEM((6, ROWS, D), F32),
            pltpu.VMEM((512, 128), F32),
            pltpu.VMEM((1, 1, D), BF16),
            pltpu.SemaphoreType.DMA((SEMS,)),
        ],
        compiler_params=pltpu.CompilerParams(
            vmem_limit_bytes=100 * 2**20,
            disable_semaphore_checks=True,
        ),
        name="adaln_decode",
    )(A_x, c, w_mod, A_wq, A_k_cache, A_v_cache, A_wo.T, B_w3, B_w4.T)
```
